```python
import os as _os
_os.environ.setdefault("JAX_PLATFORMS", "cpu")
import jax
import jax.numpy as jnp

def _softmax(x, axis=-1):
    return jax.nn.softmax(x, axis=axis)
def _gelu(x):
    return jax.nn.gelu(x, approximate=True)
def _silu(x):
    return jax.nn.silu(x)
def _sigmoid(x):
    return jax.nn.sigmoid(x)
def _layernorm(x, axis=-1, eps=1e-5):
    m = jnp.mean(x, axis=axis, keepdims=True)
    v = jnp.var(x, axis=axis, keepdims=True)
    return (x - m) / jnp.sqrt(v + eps)
def _scatter_add(tgt, idx, src, axis=0):
    return tgt.at[idx].add(src)
def _segment_sum(src, seg, n):
    return jax.ops.segment_sum(src, seg, n)
class _Rng:
    def __init__(self, key):
        self._k = key
    def _next(self):
        self._k, sub = jax.random.split(self._k)
        return sub
    def normal(self, shape):
        return jax.random.normal(self._next(), shape, dtype=jnp.bfloat16)
    def randint(self, lo, hi, shape):
        return jax.random.randint(self._next(), shape, lo, hi, dtype=jnp.int32)
    def uniform(self, shape, lo=0.0, hi=1.0):
        return jax.random.uniform(self._next(), shape, jnp.bfloat16, lo, hi)
    def permutation(self, n):
        return jax.random.permutation(self._next(), n)


kernel_name = 'sequential_preLN__ssm_conv_h3__mixer_channel_mlp__prompt'

def setup_inputs():
    _rng = _Rng(jax.random.key(int.from_bytes(__import__("os").urandom(4), "little")))
    _w = (lambda a: (lambda t: t.astype(jnp.bfloat16) if jnp.issubdtype(t.dtype, jnp.floating) else t)(jnp.asarray(a)))
    def _A_setup():
        B, S, D = 1, 2048, 448
        ks = 4
        return {
            "q": _w((lambda *s: _rng.normal(s) * 0.05)(B, S, D)),
            "k": _w((lambda *s: _rng.normal(s) * 0.05)(B, S, D)),
            "v": _w((lambda *s: _rng.normal(s) * 0.05)(B, S, D)),
            "shift_k": _w((lambda *s: _rng.normal(s) * 0.05)(D, ks) * 0.5),
            "ssm_k": _w((lambda *s: _rng.normal(s) * 0.05)(D, S) * (1.0 / S ** 0.5)),
            "ssm_D": _w((lambda *s: _rng.normal(s) * 0.05)(D)),
        }
    _A_in = _A_setup()

    def _B_setup():
        B, S, D, F = 1, 2048, 448, 1792
        return {
            "x": _w((lambda *s: _rng.normal(s) * 0.05)(B, S, D)),
            "w1": _w((lambda *s: _rng.normal(s) * 0.2)(D, F) * (D ** -0.5)),
            "b1": _w((lambda *s: _rng.normal(s) * 0.2)(F)),
            "w2": _w((lambda *s: _rng.normal(s) * 0.2)(F, D) * (F ** -0.5)),
            "b2": _w((lambda *s: _rng.normal(s) * 0.05)(D)),
        }
    _B_in = _B_setup()

    return {
        "A_q": _A_in["q"],
        "A_k": _A_in["k"],
        "A_v": _A_in["v"],
        "A_shift_k": _A_in["shift_k"],
        "A_ssm_k": _A_in["ssm_k"],
        "A_ssm_D": _A_in["ssm_D"],
        "B_x": _B_in["x"],
        "B_w1": _B_in["w1"],
        "B_b1": _B_in["b1"],
        "B_w2": _B_in["w2"],
        "B_b2": _B_in["b2"],
    }

def reference(A_q, A_k, A_v, A_shift_k, A_ssm_k, A_ssm_D, B_x, B_w1, B_b1, B_w2, B_b2):
    def _A_ref(q, k, v, shift_k, ssm_k, ssm_D):
        B, S, D = q.shape
        ks = shift_k.shape[-1]
        k_pad = jnp.pad(k, ((0, 0), (ks - 1, 0), (0, 0)))
        k_shift = jnp.zeros_like(k)
        for t in range(ks):
            k_shift = k_shift + k_pad[:, t:t + S, :] * shift_k[:, ks - 1 - t][None, None, :]
        kv = k_shift * v
        L = 2 * S
        kv_pad = jnp.pad(kv, ((0, 0), (0, S), (0, 0)))
        kf_pad = jnp.pad(ssm_k, ((0, 0), (0, S)))
        kv_f = (lambda x, axes=(-2,-1): jnp.fft.rfft2(x.astype(jnp.float32), axes=axes))(kv_pad[:, None, :, :], axes=(1, 2))
        kf_f = (lambda x, axes=(-2,-1): jnp.fft.rfft2(x.astype(jnp.float32), axes=axes))(kf_pad[:, None, :], axes=(1, 2))
        kf_f = (lambda x, *d: x.transpose(*d))(kf_f, 1, 2, 0)
        y_f = kv_f * kf_f[None, :, :, :]
        y = (lambda x, s, axes=(-2,-1): jnp.fft.irfft2(x, s=s, axes=axes).astype(jnp.bfloat16))(y_f, (1, L), axes=(1, 2))[:, 0, :S, :]
        y = y + kv * ssm_D[None, None, :]
        return q * y

    def _B_ref(x, w1, b1, w2, b2):
        y = _layernorm(x, axis=-1)
        h = _gelu(jnp.einsum("bsd,df->bsf", y, w1) + b1)
        return jnp.einsum("bsf,fd->bsd", h, w2) + b2

    x = A_q
    h = x + _A_ref(_layernorm(x, axis=-1), A_k, A_v, A_shift_k, A_ssm_k, A_ssm_D)
    h2 = h + _B_ref(_layernorm(h, axis=-1), B_w1, B_b1, B_w2, B_b2)
    return h2
```

```python
import functools
import numpy as np
import jax
import jax.numpy as jnp
from jax import lax
import jax.experimental.pallas as pl
import jax.experimental.pallas.tpu as pltpu

S, D, F, C = 2048, 448, 1792, 128
NC = S // C
DP = 512


def _dft_mats():
    n = np.arange(C, dtype=np.float64)
    k = np.arange(C, dtype=np.float64)
    ang = 2.0 * np.pi * np.outer(n, k + 0.5) / (2 * C)
    fwd = np.concatenate([np.cos(ang), -np.sin(ang)], axis=1)
    inv = np.concatenate([np.cos(ang).T, -np.sin(ang).T], axis=0) / C
    return fwd.astype(np.float32), inv.astype(np.float32)


def merge(a, b):
    wa = sum(w for w, _ in a) or 1.0
    wb = sum(w for w, _ in b) or 1.0
    out = []
    t = 0.0
    for w, f in a:
        out.append(((t) / wa, 0, f)); t += w
    t = 0.0
    for w, f in b:
        out.append(((t) / wb, 1, f)); t += w
    out.sort(key=lambda z: (z[0], z[1]))
    return [f for _, _, f in out]


def make_kernel(CPS=2, RB=16, FB=256, KB=256, mode="conv_first", bar="none", SC=1, GR=((0,0),(1,1),(2,2),(3,4),(5,6),(7,7),(8,8),(9,9),(10,10)), PAR=[8,1,1,2,2,2,2,2], ANCH=99, ANCA=-2, ANCC=-5, WS=1, PX=16, PH=8, flags=None, interpret=False):
    NS = NC // CPS
    T = CPS * C
    c0 = float(np.sqrt(2.0 / np.pi))

    def ln_t(xt):
        m = jnp.mean(xt, axis=0, keepdims=True)
        xc = xt - m
        v = jnp.mean(xc * xc, axis=0, keepdims=True)
        return xc * lax.rsqrt(v + 1e-5)

    def gelu(a):
        u = a * (c0 + (c0 * 0.044715) * (a * a))
        hx = 0.5 * a
        return hx + hx * jnp.tanh(u)

    def kernel(q_ref, k_ref, v_ref, sh_ref, hk0_ref, hk_ref, dd_ref, w1_ref, b1_ref, w2_hbm, b2_ref,
               fw_ref, gi_ref, o_ref,
               kprev, shc, dcol, b2col, w1t, xs_ref, hs_ref, hprev, ybuf, hnb, htb, gbuf, oacc,
               w1s, w2t_ref, sems):
        cp1 = pltpu.make_async_copy(w1_ref, w1s.at[0:D, :], sems.at[0])
        cp2 = pltpu.make_async_copy(w2_hbm, w2t_ref, sems.at[1])
        step = pl.program_id(0)

        def setup():
            kprev[...] = jnp.zeros_like(kprev)
            xs_ref[0:CPS] = jnp.zeros((CPS, 3, D + PX, C), jnp.float32)
            shf = sh_ref[...].astype(jnp.float32)
            for j in range(4):
                shc[j] = jnp.broadcast_to(shf[j:j + 1, :], (C, D)).T
            dcol[...] = jnp.broadcast_to(dd_ref[...].astype(jnp.float32).reshape(1, D), (C, D)).T
            b2col[...] = jnp.broadcast_to(b2_ref[...].astype(jnp.float32).reshape(1, D), (C, D)).T
            cp1.start()
            cp2.start()
            w1s[D:DP, :] = jnp.concatenate(
                [b1_ref[...].reshape(1, F), jnp.zeros((DP - D - 1, F), jnp.bfloat16)], axis=0)
            row = lax.broadcasted_iota(jnp.int32, (DP - D, T), 0)
            for p in range(2):
                hnb[p, D:DP, :] = jnp.where(row == 0, 1.0, 0.0).astype(jnp.bfloat16)

        def stageA_x(g, c):
            I = (g + 1) * CPS + c
            lane2 = lax.broadcasted_iota(jnp.int32, (D, C), 1)
            cs = slice(c * C, (c + 1) * C)
            kc = k_ref[:, cs].astype(jnp.float32)
            kp = kprev[...]
            kprev[...] = kc
            ks = kc * shc[0]
            for j in range(1, 4):
                ks = ks + pltpu.roll(jnp.where(lane2 >= C - j, kp, kc), j, 1) * shc[j]
            kvt = (ks * v_ref[:, cs].astype(jnp.float32)).astype(jnp.bfloat16)
            X = jnp.dot(kvt, fw_ref[...], preferred_element_type=jnp.float32)
            xr, xi = X[:, :C], X[:, C:]
            xs_ref[I, 0, 0:D, :] = xr
            xs_ref[I, 1, 0:D, :] = xi
            xs_ref[I, 2, 0:D, :] = xr + xi
            note('a', xr + xi)

        def stageA_h(g, c):
            I = g * CPS + c
            cs = slice(c * C, (c + 1) * C)
            lane = lax.broadcasted_iota(jnp.int32, (1, C), 1)
            sgn = jnp.where(lane % 2 == 0, 1.0, -1.0).astype(jnp.float32)
            H = jnp.dot((hk0_ref if isinstance(g, int) and g == 0 else hk_ref)[:, cs], fw_ref[...], preferred_element_type=jnp.float32)
            hr, hi = H[:, :C], H[:, C:]
            if isinstance(I, int) and I == 0:
                hr = hr + dcol[...]
                pr, pi = hr, hi
            else:
                pr = hr - sgn * hprev[1]
                pi = hi + sgn * hprev[0]
            hprev[0] = hr
            hprev[1] = hi
            hs_ref[I, 0, 0:D, :] = pr
            hs_ref[I, 1, 0:D, :] = pi - pr
            hs_ref[I, 2, 0:D, :] = pr + pi
            note('a', pr + pi)

        dep = {}

        def stageB(g, gm, r):
            res = [[None] * 3 for _ in range(CPS)]
            npar = PAR if isinstance(PAR, int) else PAR[gm]
            for t in range(3):
                xt = (2, 0, 1)[t]
                for hf in range(RB // 8):
                    rs = slice(r * RB + hf * 8, r * RB + hf * 8 + 8)
                    ch = dep["n"] % npar
                    dep["n"] += 1
                    z = dep.get(ch)
                    acc = [None] * CPS
                    hc = {}
                    xv = xs_ref.at[pl.ds((g - gm + 1) * CPS, (gm + 1) * CPS)]
                    for i in range(gm * CPS + CPS):
                        x = xv[i, xt, rs, :]
                        for c in range(CPS):
                            dl = gm * CPS + c - i
                            if dl < 0:
                                continue
                            if dl not in hc:
                                hc[dl] = hs_ref[dl, t, rs, :]
                            p = x * hc[dl]
                            if acc[c] is None:
                                if z is not None:
                                    p = pltpu.bitcast(pltpu.bitcast(p, jnp.int32) | z, jnp.float32)
                                acc[c] = p
                            else:
                                acc[c] = acc[c] + p
                    dep[ch] = pltpu.bitcast(acc[-1], jnp.int32) & dep["m"]
                    for c in range(CPS):
                        res[c][t] = acc[c] if hf == 0 else jnp.concatenate([res[c][t], acc[c]], axis=0)
            rs = slice(r * RB, (r + 1) * RB)
            for c in range(CPS):
                ybuf[g % 2, c, rs, 0:C] = (res[c][0] - res[c][2]).astype(jnp.bfloat16)
                ybuf[g % 2, c, rs, C:] = (res[c][0] + res[c][1]).astype(jnp.bfloat16)

        def stageC(g, c):
            cs = slice(c * C, (c + 1) * C)
            yt = jnp.dot(ybuf[g % 2, c], gi_ref[...], preferred_element_type=jnp.float32)
            xt = q_ref[:, cs].astype(jnp.float32)
            ht = xt + ln_t(xt) * yt
            hnb[g % 2, 0:D, cs] = ln_t(ht).astype(jnp.bfloat16)
            htb[g % 2, :, cs] = ht + b2col[...]
            note('c', ln_t(ht))

        def note(k, v):
            for r in range(0, v.shape[0], 64):
                b = pltpu.bitcast(v[r + 48:r + 56, 0:128], jnp.int32) & dep['m']
                dep[k] = b if k not in dep else dep[k] | b

        def gate(lhs, on, k):
            if not on or k not in dep:
                return lhs
            z = dep[k]
            top = pltpu.bitcast(lhs[0:16, :], jnp.int32) | jnp.concatenate([z] * (lhs.shape[1] // 128), axis=1)
            return jnp.concatenate([pltpu.bitcast(top, jnp.bfloat16), lhs[16:, :]], axis=0)

        def mm1(g, f):
            fs = slice(f * FB, (f + 1) * FB)
            a = jnp.dot(gate(gate(w1t[fs, :], f - F // FB == ANCA, 'a'), f - F // FB == ANCC, 'c'), hnb[g % 2], preferred_element_type=jnp.float32)
            gbuf[fs, :] = gelu(a).astype(jnp.bfloat16)

        def mm2(g, j):
            ks_ = slice(j * KB, (j + 1) * KB)
            o = jnp.dot(gate(gate(gate(w2t_ref[:, ks_], j == ANCH, 0), j == ANCA, 'a'), j == ANCC, 'c'), gbuf[ks_, :], preferred_element_type=jnp.float32)
            if j == 0:
                o = o + htb[g % 2]
            else:
                o = o + oacc[...]
            if j == F // KB - 1:
                o_ref[...] = o.astype(o_ref.dtype)
            else:
                oacc[...] = o

        def do_step(s0, s):
            sd = s if s0 == s else step
            P = functools.partial
            dep.clear(); dep['n'] = 0
            dep['m'] = jnp.full((8, 128), step >> 8, jnp.int32)
            conv, mlp = [], []
            if s == 0:
                setup()
            if s == WS:
                cp1.wait()
                w1t[...] = w1s[...].T
            if s == 2:
                pass
            if False:
                cp2.wait()
            if 1 <= s <= NS:
                nr = D // RB
                for r in range(nr):
                    conv.append((0.5 / nr, P(stageB, sd - 1, s - 1, r)))
            if 2 <= s <= NS + 1:
                for c in range(CPS):
                    conv.append((0.1, P(stageC, sd - 2, c)))
            if s == 0:
                for c in range(CPS):
                    conv.append((0.05, P(stageA_h, 0, c)))
            for c in range(CPS):
                if s + 1 < NS:
                    conv.append((0.05, P(stageA_h, sd + 1, c)))
                if s < NS:
                    conv.append((0.05, P(stageA_x, sd, c)))
            if s >= 3:
                for f in range(F // FB):
                    mlp.append((FB * 4, P(mm1, sd - 3, f)))
                for j in range(F // KB):
                    mlp.append((KB * 3.5, P(mm2, sd - 3, j)))
            if mode == "merge":
                seq = merge(mlp, conv)
            elif mode == "mlp_first":
                seq = [f for _, f in mlp] + [f for _, f in conv]
            elif mode == "conv_first":
                seq = [f for _, f in conv] + [f for _, f in mlp]
                nb = D // RB if 1 <= s <= NS else 0
                cv = [f for _, f in conv]; ml = [f for _, f in mlp]; cut = F // FB + 1
                seq = cv[:nb] + ml[:cut] + cv[nb:] + ml[cut:]
            if s == 2:
                seq = seq + [cp2.wait]
            for n, f in enumerate(seq):
                if bar == "scope":
                    with jax.named_scope("p%d" % n):
                        f()
                elif bar == "touch":
                    f()
                    pltpu.touch((ybuf, gbuf, w1t, xs_ref, hs_ref))
                else:
                    f()

        for s0, s1 in GR:
            pl.when((step >= s0) & (step <= s1))(functools.partial(do_step, s0, s1))

    fwd_np, inv_np = _dft_mats()

    @jax.jit
    def run(A_q, A_k, A_v, A_shift_k, A_ssm_k, A_ssm_D, B_x, B_w1, B_b1, B_w2, B_b2):
        del B_x
        tok = pl.BlockSpec((D, T), lambda i: (0, jnp.minimum(i, NS - 1)))
        otok = pl.BlockSpec((D, T), lambda i: (0, jnp.maximum(i - 2 - SC, 0)))
        full = lambda shape: pl.BlockSpec(shape, lambda i: (0,) * len(shape))
        out = pl.pallas_call(
            kernel,
            grid=(NS + 2 + SC,),
            in_specs=[pl.BlockSpec((D, T), lambda i: (0, jnp.clip(i - 1 - SC, 0, NS - 1))), tok, tok, full((4, D)), pl.BlockSpec((D, T), lambda i: (0, 0)), pl.BlockSpec((D, T), lambda i: (0, jnp.minimum(i + 1, NS - 1))), full((D,)),
                      pl.BlockSpec(memory_space=pl.ANY), full((F,)), pl.BlockSpec(memory_space=pl.ANY), full((D,)), full((C, 2 * C)), full((2 * C, C))],
            out_specs=otok,
            out_shape=jax.ShapeDtypeStruct((D, S), jnp.bfloat16),
            scratch_shapes=[
                pltpu.VMEM((D, C), jnp.float32),
                pltpu.VMEM((4, D, C), jnp.float32),
                pltpu.VMEM((D, C), jnp.float32),
                pltpu.VMEM((D, C), jnp.float32),
                pltpu.VMEM((F, DP), jnp.bfloat16),
                pltpu.VMEM((NC + CPS, 3, D + PX, C), jnp.float32),
                pltpu.VMEM((NC, 3, D + PH, C), jnp.float32),
                pltpu.VMEM((2, D, C), jnp.float32),
                pltpu.VMEM((2, CPS, D, 2 * C), jnp.bfloat16),
                pltpu.VMEM((2, DP, T), jnp.bfloat16),
                pltpu.VMEM((2, D, T), jnp.float32),
                pltpu.VMEM((F, T), jnp.bfloat16),
                pltpu.VMEM((D, T), jnp.float32),
                pltpu.VMEM((DP, F), jnp.bfloat16),
                pltpu.VMEM((D, F), jnp.bfloat16),
                pltpu.SemaphoreType.DMA((2,)),
            ],
            compiler_params=pltpu.CompilerParams(
                flags=flags, dimension_semantics=("arbitrary",), vmem_limit_bytes=100 * 1024 * 1024),
            interpret=interpret,
        )(A_q[0].T, A_k[0].T, A_v[0].T, A_shift_k.T, A_ssm_k, A_ssm_k, A_ssm_D,
          B_w1, B_b1, B_w2.T, B_b2, jnp.asarray(fwd_np, jnp.bfloat16), jnp.asarray(inv_np, jnp.bfloat16))
        return out.T[None]

    return run


pallas_sequential_preLN__ssm_conv_h3__mixer_channel_mlp__prompt_kernel = make_kernel(
    KB=128, ANCA=-4, flags={"XLA_TPU_EVENLY_DISTRIBUTE_CRITICAL_NODES": True})
```
